```python
import os as _os
_os.environ.setdefault("JAX_PLATFORMS", "cpu")
import jax
import jax.numpy as jnp

def _softmax(x, axis=-1):
    return jax.nn.softmax(x, axis=axis)
def _gelu(x):
    return jax.nn.gelu(x, approximate=True)
def _silu(x):
    return jax.nn.silu(x)
def _sigmoid(x):
    return jax.nn.sigmoid(x)
def _layernorm(x, axis=-1, eps=1e-5):
    m = jnp.mean(x, axis=axis, keepdims=True)
    v = jnp.var(x, axis=axis, keepdims=True)
    return (x - m) / jnp.sqrt(v + eps)
def _scatter_add(tgt, idx, src, axis=0):
    return tgt.at[idx].add(src)
def _segment_sum(src, seg, n):
    return jax.ops.segment_sum(src, seg, n)
class _Rng:
    def __init__(self, key):
        self._k = key
    def _next(self):
        self._k, sub = jax.random.split(self._k)
        return sub
    def normal(self, shape):
        return jax.random.normal(self._next(), shape, dtype=jnp.bfloat16)
    def randint(self, lo, hi, shape):
        return jax.random.randint(self._next(), shape, lo, hi, dtype=jnp.int32)
    def uniform(self, shape, lo=0.0, hi=1.0):
        return jax.random.uniform(self._next(), shape, jnp.bfloat16, lo, hi)
    def permutation(self, n):
        return jax.random.permutation(self._next(), n)


kernel_name = 'parallel_sum__ssm_conv_h3__dense_activation_silu__prompt'

def setup_inputs():
    _rng = _Rng(jax.random.key(int.from_bytes(__import__("os").urandom(4), "little")))
    _w = (lambda a: (lambda t: t.astype(jnp.bfloat16) if jnp.issubdtype(t.dtype, jnp.floating) else t)(jnp.asarray(a)))
    def _A_setup():
        B, S, D = 1, 2048, 448
        ks = 4
        return {
            "q": _w((lambda *s: _rng.normal(s) * 0.05)(B, S, D)),
            "k": _w((lambda *s: _rng.normal(s) * 0.2)(B, S, D)),
            "v": _w((lambda *s: _rng.normal(s) * 0.2)(B, S, D)),
            "shift_k": _w((lambda *s: _rng.normal(s) * 0.2)(D, ks) * 0.5),
            "ssm_k": _w((lambda *s: _rng.normal(s) * 0.2)(D, S) * (1.0 / S ** 0.5)),
            "ssm_D": _w((lambda *s: _rng.normal(s) * 0.2)(D)),
        }
    _A_in = _A_setup()

    def _B_setup():
        B, S, D, F = 1, 2048, 448, 1792
        return {
            "x": _w((lambda *s: _rng.normal(s) * 0.05)(B, S, D)),
            "w1": _w((lambda *s: _rng.normal(s) * 0.05)(D, F) * (D ** -0.5)),
            "w2": _w((lambda *s: _rng.normal(s) * 0.05)(F, D) * (F ** -0.5)),
        }
    _B_in = _B_setup()

    return {
        "A_q": _A_in["q"],
        "A_k": _A_in["k"],
        "A_v": _A_in["v"],
        "A_shift_k": _A_in["shift_k"],
        "A_ssm_k": _A_in["ssm_k"],
        "A_ssm_D": _A_in["ssm_D"],
        "B_x": _B_in["x"],
        "B_w1": _B_in["w1"],
        "B_w2": _B_in["w2"],
    }

def reference(A_q, A_k, A_v, A_shift_k, A_ssm_k, A_ssm_D, B_x, B_w1, B_w2):
    def _A_ref(q, k, v, shift_k, ssm_k, ssm_D):
        B, S, D = q.shape
        ks = shift_k.shape[-1]
        k_pad = jnp.pad(k, ((0, 0), (ks - 1, 0), (0, 0)))
        k_shift = jnp.zeros_like(k)
        for t in range(ks):
            k_shift = k_shift + k_pad[:, t:t + S, :] * shift_k[:, ks - 1 - t][None, None, :]
        kv = k_shift * v
        L = 2 * S
        kv_pad = jnp.pad(kv, ((0, 0), (0, S), (0, 0)))
        kf_pad = jnp.pad(ssm_k, ((0, 0), (0, S)))
        kv_f = (lambda x, axes=(-2,-1): jnp.fft.rfft2(x.astype(jnp.float32), axes=axes))(kv_pad[:, None, :, :], axes=(1, 2))
        kf_f = (lambda x, axes=(-2,-1): jnp.fft.rfft2(x.astype(jnp.float32), axes=axes))(kf_pad[:, None, :], axes=(1, 2))
        kf_f = (lambda x, *d: x.transpose(*d))(kf_f, 1, 2, 0)
        y_f = kv_f * kf_f[None, :, :, :]
        y = (lambda x, s, axes=(-2,-1): jnp.fft.irfft2(x, s=s, axes=axes).astype(jnp.bfloat16))(y_f, (1, L), axes=(1, 2))[:, 0, :S, :]
        y = y + kv * ssm_D[None, None, :]
        return q * y

    def _B_ref(x, w1, w2):
        h = jnp.einsum("bsd,df->bsf", x, w1)
        h = _silu(h)
        out = jnp.einsum("bsf,fd->bsd", h, w2)
        return out

    x = A_q
    xn = _layernorm(x, axis=-1)
    return x + _A_ref(xn, A_k, A_v, A_shift_k, A_ssm_k, A_ssm_D) + _B_ref(xn, B_w1, B_w2)
```

```python
import functools

import numpy as np
import jax
import jax.numpy as jnp
from jax import lax
import jax.experimental.pallas as pl
import jax.experimental.pallas.tpu as pltpu

f32 = jnp.float32
bf16 = jnp.bfloat16

C = 128


def _dft_consts(c):
    n = np.arange(c, dtype=np.float64)
    f = np.arange(c, dtype=np.float64)
    th = np.pi * np.outer(2 * f + 1, n) / (2 * c)
    fm = np.concatenate([np.cos(th), -np.sin(th)], 0)
    n2 = np.arange(2 * c, dtype=np.float64)
    th2 = np.pi * np.outer(n2, 2 * f + 1) / (2 * c)
    gm = np.concatenate([np.cos(th2), -np.sin(th2)], 1) / c
    g = np.concatenate([gm[:c], gm[c:]], 1)
    return fm, g


def _kernel(q_ref, k_ref, v_ref, sk_ref, ssmk_ref, sd_ref, w1_ref, w2_ref,
            f_ref, g_ref, o_ref,
            xs_ref, ks_ref, pprev_ref, kcarry_ref, *, nb, d):
    i = pl.program_id(0)

    @pl.when(i == 0)
    def _():
        fm = f_ref[...]
        for m in range(nb):
            kb = ssmk_ref[:, m * C:(m + 1) * C]
            ks_ref[m] = lax.dot_general(
                fm, kb, (((1,), (1,)), ((), ())), preferred_element_type=f32)
        pprev_ref[...] = jnp.zeros_like(pprev_ref)
        kcarry_ref[...] = jnp.zeros_like(kcarry_ref)

    k = k_ref[...].astype(f32)
    kext = jnp.concatenate([kcarry_ref[...], k], axis=0)
    kcarry_ref[...] = k[C - 8:, :]
    sk = sk_ref[...].astype(f32)
    kshift = k * sk[0:1, :]
    for l in range(1, 4):
        kshift = kshift + kext[8 - l:8 - l + C, :] * sk[l:l + 1, :]
    kv = kshift * v_ref[...].astype(f32)

    xs_ref[i] = jnp.dot(f_ref[...], kv.astype(bf16), preferred_element_type=f32)

    RC = 16
    pcs = []
    for rc in range(C // RC):
        r0 = rc * RC

        def body(j, acc, r0=r0):
            ar, ai = acc
            xr = xs_ref[j, r0:r0 + RC, :]
            xi = xs_ref[j, C + r0:C + r0 + RC, :]
            kr = ks_ref[i - j, r0:r0 + RC, :]
            ki = ks_ref[i - j, C + r0:C + r0 + RC, :]
            ar = ar + (xr * kr - xi * ki)
            ai = ai + (xr * ki + xi * kr)
            return ar, ai

        z = jnp.zeros((RC, d), f32)
        ar, ai = lax.fori_loop(0, i + 1, body, (z, z))
        pcs.append((ar.astype(bf16), ai.astype(bf16)))
    p = jnp.concatenate([a for a, _ in pcs] + [b for _, b in pcs], axis=0)
    pcat = jnp.concatenate([p, pprev_ref[...]], axis=0)
    pprev_ref[...] = p
    y = jnp.dot(g_ref[...], pcat, preferred_element_type=f32)
    y = y + kv * sd_ref[...].astype(f32)

    x = q_ref[...].astype(f32)
    mu = jnp.mean(x, axis=-1, keepdims=True)
    xc = x - mu
    var = jnp.mean(xc * xc, axis=-1, keepdims=True)
    xn = xc * lax.rsqrt(var + 1e-5)

    h = jnp.dot(xn.astype(bf16), w1_ref[...], preferred_element_type=f32)
    h = h * jax.nn.sigmoid(h)
    ffn = jnp.dot(h.astype(bf16), w2_ref[...], preferred_element_type=f32)

    o_ref[...] = (x + xn * y + ffn).astype(o_ref.dtype)


@jax.jit
def pallas_parallel_sum__ssm_conv_h3__dense_activation_silu__prompt_kernel(
    A_q: jax.Array,
    A_k: jax.Array,
    A_v: jax.Array,
    A_shift_k: jax.Array,
    A_ssm_k: jax.Array,
    A_ssm_D: jax.Array,
    B_x: jax.Array,
    B_w1: jax.Array,
    B_w2: jax.Array,
):
    B, S, D = A_q.shape
    F = B_w1.shape[1]
    nb = S // C
    q = A_q.reshape(S, D)
    k = A_k.reshape(S, D)
    v = A_v.reshape(S, D)
    sk = A_shift_k.T
    sd = A_ssm_D.reshape(1, D)
    fm, g = _dft_consts(C)
    fm = jnp.asarray(fm, dtype=bf16)
    g = jnp.asarray(g, dtype=bf16)

    full = lambda shape: pl.BlockSpec(shape, lambda i: (0,) * len(shape))
    row = pl.BlockSpec((C, D), lambda i: (i, 0))
    out = pl.pallas_call(
        functools.partial(_kernel, nb=nb, d=D),
        grid=(nb,),
        in_specs=[row, row, row, full((4, D)), full((D, S)), full((1, D)),
                  full((D, F)), full((F, D)), full((2 * C, C)), full((C, 4 * C))],
        out_specs=row,
        out_shape=jax.ShapeDtypeStruct((S, D), A_q.dtype),
        scratch_shapes=[
            pltpu.VMEM((nb, 2 * C, D), f32),
            pltpu.VMEM((nb, 2 * C, D), f32),
            pltpu.VMEM((2 * C, D), bf16),
            pltpu.VMEM((8, D), f32),
        ],
        compiler_params=pltpu.CompilerParams(
            dimension_semantics=("arbitrary",),
            vmem_limit_bytes=100 * 1024 * 1024,
        ),
    )(q, k, v, sk, A_ssm_k, sd, B_w1, B_w2, fm, g)
    return out.reshape(B, S, D)
```

```python
import functools

import numpy as np
import jax
import jax.numpy as jnp
from jax import lax
import jax.experimental.pallas as pl
import jax.experimental.pallas.tpu as pltpu

f32 = jnp.float32
bf16 = jnp.bfloat16

C = 128


def _dft_consts(c):
    n = np.arange(c, dtype=np.float64)
    f = np.arange(c, dtype=np.float64)
    th = np.pi * np.outer(2 * f + 1, n) / (2 * c)
    fm = np.concatenate([np.cos(th), -np.sin(th)], 0)
    n2 = np.arange(2 * c, dtype=np.float64)
    th2 = np.pi * np.outer(n2, 2 * f + 1) / (2 * c)
    gm = np.concatenate([np.cos(th2), -np.sin(th2)], 1) / c
    g = np.concatenate([gm[:c], gm[c:]], 1)
    return fm.T, g.T


def _kernel(q_ref, k_ref, v_ref, sk_ref, ssmk_ref, sd_ref, w1_ref, w2t_ref,
            f_ref, g_ref, o_ref,
            xs_ref, ks_ref, pprev_ref, kprev_ref, w1t_ref, *, nb, d):
    i = pl.program_id(0)

    @pl.when(i == 0)
    def _():
        fm = f_ref[...]
        for m in range(nb):
            kb = ssmk_ref[:, m * C:(m + 1) * C]
            ks_ref[m] = jnp.dot(kb, fm, preferred_element_type=f32)
        pprev_ref[...] = jnp.zeros_like(pprev_ref)
        kprev_ref[...] = jnp.zeros_like(kprev_ref)
        w1t_ref[...] = w1_ref[...].T

    k = k_ref[...].astype(f32)
    kp = kprev_ref[...]
    kprev_ref[...] = k
    sk = sk_ref[...].astype(f32)
    lane = lax.broadcasted_iota(jnp.int32, (d, C), 1)
    kshift = k * sk[:, 0:1]
    for l in range(1, 4):
        sh = jnp.where(lane < l, pltpu.roll(kp, l, 1), pltpu.roll(k, l, 1))
        kshift = kshift + sh * sk[:, l:l + 1]
    kv = kshift * v_ref[...].astype(f32)

    xs_ref[i] = jnp.dot(kv.astype(bf16), f_ref[...], preferred_element_type=f32)

    RC = 32
    pcs = []
    for rc in range(d // RC):
        r0 = rc * RC

        def body(j, acc, r0=r0):
            ar, ai = acc
            xr = xs_ref[j, r0:r0 + RC, 0:C]
            xi = xs_ref[j, r0:r0 + RC, C:2 * C]
            kr = ks_ref[i - j, r0:r0 + RC, 0:C]
            ki = ks_ref[i - j, r0:r0 + RC, C:2 * C]
            ar = ar + (xr * kr - xi * ki)
            ai = ai + (xr * ki + xi * kr)
            return ar, ai

        z = jnp.zeros((RC, C), f32)
        ar, ai = lax.fori_loop(0, i + 1, body, (z, z))
        pcs.append(jnp.concatenate([ar, ai], axis=1).astype(bf16))
    p = jnp.concatenate(pcs, axis=0)
    pcat = jnp.concatenate([p, pprev_ref[...]], axis=1)
    pprev_ref[...] = p
    y = jnp.dot(pcat, g_ref[...], preferred_element_type=f32)
    y = y + kv * sd_ref[...].astype(f32)

    x = q_ref[...].astype(f32)
    mu = jnp.mean(x, axis=0, keepdims=True)
    xc = x - mu
    var = jnp.mean(xc * xc, axis=0, keepdims=True)
    xn = xc * lax.rsqrt(var + 1e-5)

    h = jnp.dot(w1t_ref[...], xn.astype(bf16), preferred_element_type=f32)
    h = h * jax.nn.sigmoid(h)
    ffn = jnp.dot(w2t_ref[...], h.astype(bf16), preferred_element_type=f32)

    o_ref[...] = (x + xn * y + ffn).astype(o_ref.dtype)


@jax.jit
def pallas_parallel_sum__ssm_conv_h3__dense_activation_silu__prompt_kernel(
    A_q: jax.Array,
    A_k: jax.Array,
    A_v: jax.Array,
    A_shift_k: jax.Array,
    A_ssm_k: jax.Array,
    A_ssm_D: jax.Array,
    B_x: jax.Array,
    B_w1: jax.Array,
    B_w2: jax.Array,
):
    B, S, D = A_q.shape
    F = B_w1.shape[1]
    nb = S // C
    q = A_q.reshape(S, D).T
    k = A_k.reshape(S, D).T
    v = A_v.reshape(S, D).T
    sd = A_ssm_D.reshape(D, 1)
    w2t = B_w2.T
    fm, g = _dft_consts(C)
    fm = jnp.asarray(fm, dtype=bf16)
    g = jnp.asarray(g, dtype=bf16)

    full = lambda shape: pl.BlockSpec(shape, lambda i: (0,) * len(shape))
    col = pl.BlockSpec((D, C), lambda i: (0, i))
    out = pl.pallas_call(
        functools.partial(_kernel, nb=nb, d=D),
        grid=(nb,),
        in_specs=[col, col, col, full((D, 4)), full((D, S)), full((D, 1)),
                  full((D, F)), full((D, F)), full((C, 2 * C)), full((4 * C, C))],
        out_specs=col,
        out_shape=jax.ShapeDtypeStruct((D, S), A_q.dtype),
        scratch_shapes=[
            pltpu.VMEM((nb, D, 2 * C), f32),
            pltpu.VMEM((nb, D, 2 * C), f32),
            pltpu.VMEM((D, 2 * C), bf16),
            pltpu.VMEM((D, C), f32),
            pltpu.VMEM((F, D), bf16),
        ],
        compiler_params=pltpu.CompilerParams(
            dimension_semantics=("arbitrary",),
            vmem_limit_bytes=100 * 1024 * 1024,
        ),
    )(q, k, v, A_shift_k, A_ssm_k, sd, B_w1, w2t, fm, g)
    return out.T.reshape(B, S, D)
```

```python
import functools

import numpy as np
import jax
import jax.numpy as jnp
from jax import lax
import jax.experimental.pallas as pl
import jax.experimental.pallas.tpu as pltpu

f32 = jnp.float32
bf16 = jnp.bfloat16

C = 128
T = 256
RC = 32
PR = 64


def _dft_consts(c):
    n = np.arange(c, dtype=np.float64)
    f = np.arange(c, dtype=np.float64)
    th = np.pi * np.outer(2 * f + 1, n) / (2 * c)
    fm = np.concatenate([np.cos(th), -np.sin(th)], 0)
    gm = np.concatenate([np.cos(th.T), -np.sin(th.T)], 1) / c
    return fm.T, gm.T


def _schedule(ns):
    tab = []
    for t in range(ns):
        for j in range(2 * t + 2):
            tab.append((t, j))
    per = len(tab) // ns
    assert per * ns == len(tab)
    return np.array(tab, dtype=np.int32).T.copy(), per


def _kernel(tab_ref, q_ref, k0_ref, v0_ref, k_ref, v_ref, sk_ref, sd_ref, f_ref, g_ref,
            ssmk_hbm, w1_hbm, w2t_hbm, o_ref,
            xs_ref, ks_ref, pacc_ref, kvb_ref, kext_ref, w1t_ref, tap_ref, kvd_ref,
            ssmk_ref, w1_ref, w2t_ref, sems, *, nb, d, ns, per):
    s = pl.program_id(0)

    cp_ssmk = pltpu.make_async_copy(ssmk_hbm, ssmk_ref, sems.at[0])
    cp_w1 = pltpu.make_async_copy(w1_hbm, w1_ref, sems.at[1])
    cp_w2 = pltpu.make_async_copy(w2t_hbm, w2t_ref, sems.at[2])

    def process_block(b, kr, vr):
        for c in range(d // PR):
            rows = slice(c * PR, (c + 1) * PR)
            kb = kr[rows, :]
            ku = pltpu.bitcast(
                jnp.concatenate([kext_ref[rows, :], kb], axis=1), jnp.uint32)
            kext_ref[rows, :] = kb[:, T - C:]
            kshift = kb.astype(f32) * jnp.concatenate(
                [tap_ref[0, rows, :]] * (T // C), axis=1)
            for l in range(1, 4):
                sh = pltpu.bitcast(pltpu.roll(ku, l, 1)[:, C:], bf16).astype(f32)
                kshift = kshift + sh * jnp.concatenate(
                    [tap_ref[l, rows, :]] * (T // C), axis=1)
            kv = kshift * vr[rows, :].astype(f32)
            kvd_ref[b, rows, :] = kv * sd_ref[rows, :].astype(f32)
            kvb_ref[rows, :] = kv.astype(bf16)
        xs_ref[2 * b] = jnp.dot(kvb_ref[:, :C], f_ref[...], preferred_element_type=f32)
        xs_ref[2 * b + 1] = jnp.dot(kvb_ref[:, C:], f_ref[...], preferred_element_type=f32)

    @pl.when(s == 0)
    def _():
        cp_ssmk.start()
        cp_w1.start()
        cp_w2.start()
        kext_ref[...] = jnp.zeros_like(kext_ref)
        pacc_ref[...] = jnp.zeros_like(pacc_ref)
        sk = sk_ref[...].astype(f32)
        for l in range(4):
            tap_ref[l] = jnp.broadcast_to(sk[:, l:l + 1], (d, C))
        process_block(0, k0_ref, v0_ref)

    @pl.when(s < ns - 1)
    def _():
        process_block(s + 1, k_ref, v_ref)

    @pl.when(s == 0)
    def _():
        cp_ssmk.wait()
        fm = f_ref[...]
        ks_ref[0] = jnp.zeros((d, 2 * C), f32)
        lane = lax.broadcasted_iota(jnp.int32, (1, C), 1)
        sig = jnp.where(lane % 2 == 0, 1.0, -1.0).astype(f32)
        pr = pi = None
        for m in range(nb):
            kbm = ssmk_ref[:, m * C:(m + 1) * C]
            km = jnp.dot(kbm, fm, preferred_element_type=f32)
            kr, ki = km[:, :C], km[:, C:]
            if m == 0:
                ks_ref[m + 1] = km
            else:
                ks_ref[m + 1, :, 0:C] = kr - sig * pi
                ks_ref[m + 1, :, C:2 * C] = ki + sig * pr
            pr, pi = kr, ki
        cp_w1.wait()
        w1t_ref[...] = w1_ref[...].T
        cp_w2.wait()

    x = q_ref[...].astype(f32)
    mu = jnp.mean(x, axis=0, keepdims=True)
    xc = x - mu
    var = jnp.mean(xc * xc, axis=0, keepdims=True)
    xn = xc * lax.rsqrt(var + 1e-5)
    xnb = xn.astype(bf16)

    for u in range(per):
        n = s * per + u
        t = tab_ref[0, n]
        j = tab_ref[1, n]
        m0 = 2 * t - j + 1
        for rc in range(d // RC):
            r0 = rc * RC
            xr = xs_ref[j, r0:r0 + RC, 0:C]
            xi = xs_ref[j, r0:r0 + RC, C:2 * C]
            k0r = ks_ref[m0, r0:r0 + RC, 0:C]
            k0i = ks_ref[m0, r0:r0 + RC, C:2 * C]
            k1r = ks_ref[m0 + 1, r0:r0 + RC, 0:C]
            k1i = ks_ref[m0 + 1, r0:r0 + RC, C:2 * C]
            pacc_ref[2 * t, r0:r0 + RC, 0:C] += xr * k0r - xi * k0i
            pacc_ref[2 * t, r0:r0 + RC, C:2 * C] += xr * k0i + xi * k0r
            pacc_ref[2 * t + 1, r0:r0 + RC, 0:C] += xr * k1r - xi * k1i
            pacc_ref[2 * t + 1, r0:r0 + RC, C:2 * C] += xr * k1i + xi * k1r

    h = jnp.dot(w1t_ref[...], xnb, preferred_element_type=f32)
    hh = 0.5 * h
    h = (hh + hh * jnp.tanh(hh)).astype(bf16)
    ffn = jnp.dot(w2t_ref[...], h, preferred_element_type=f32)

    y0 = jnp.dot(pacc_ref[2 * s].astype(bf16), g_ref[...], preferred_element_type=f32)
    y1 = jnp.dot(pacc_ref[2 * s + 1].astype(bf16), g_ref[...], preferred_element_type=f32)
    y = jnp.concatenate([y0, y1], axis=1) + kvd_ref[s]
    o_ref[...] = (x + xn * y + ffn).astype(o_ref.dtype)


@jax.jit
def pallas_parallel_sum__ssm_conv_h3__dense_activation_silu__prompt_kernel(
    A_q: jax.Array,
    A_k: jax.Array,
    A_v: jax.Array,
    A_shift_k: jax.Array,
    A_ssm_k: jax.Array,
    A_ssm_D: jax.Array,
    B_x: jax.Array,
    B_w1: jax.Array,
    B_w2: jax.Array,
):
    B, S, D = A_q.shape
    F = B_w1.shape[1]
    nb = S // C
    ns = S // T
    q = A_q.reshape(S, D).T
    k = A_k.reshape(S, D).T
    v = A_v.reshape(S, D).T
    sd = A_ssm_D.reshape(D, 1)
    w2t = B_w2.T
    fm, g = _dft_consts(C)
    fm = jnp.asarray(fm, dtype=bf16)
    g = jnp.asarray(g, dtype=bf16)
    tab, per = _schedule(ns)
    tab = jnp.asarray(tab)

    full = lambda shape: pl.BlockSpec(shape, lambda i: (0,) * len(shape))
    col = pl.BlockSpec((D, T), lambda i: (0, i))
    col0 = pl.BlockSpec((D, T), lambda i: (0, 0))
    coln = pl.BlockSpec((D, T), lambda i: (0, jnp.minimum(i + 1, ns - 1)))
    hbm = pl.BlockSpec(memory_space=pl.ANY)
    out = pl.pallas_call(
        functools.partial(_kernel, nb=nb, d=D, ns=ns, per=per),
        grid=(ns,),
        in_specs=[pl.BlockSpec(memory_space=pltpu.SMEM),
                  col, col0, col0, coln, coln, full((D, 4)), full((D, 1)),
                  full((C, 2 * C)), full((2 * C, C)), hbm, hbm, hbm],
        out_specs=col,
        out_shape=jax.ShapeDtypeStruct((D, S), A_q.dtype),
        scratch_shapes=[
            pltpu.VMEM((nb, D, 2 * C), f32),
            pltpu.VMEM((nb + 1, D, 2 * C), f32),
            pltpu.VMEM((nb, D, 2 * C), f32),
            pltpu.VMEM((D, T), bf16),
            pltpu.VMEM((D, C), bf16),
            pltpu.VMEM((F, D), bf16),
            pltpu.VMEM((4, D, C), f32),
            pltpu.VMEM((ns, D, T), f32),
            pltpu.VMEM((D, S), bf16),
            pltpu.VMEM((D, F), bf16),
            pltpu.VMEM((D, F), bf16),
            pltpu.SemaphoreType.DMA((3,)),
        ],
        compiler_params=pltpu.CompilerParams(
            dimension_semantics=("arbitrary",),
            vmem_limit_bytes=100 * 1024 * 1024,
        ),
    )(tab, q, k, v, k, v, A_shift_k, sd, fm, g, A_ssm_k, B_w1, w2t)
    return out.T.reshape(B, S, D)
```

```python
import functools

import numpy as np
import jax
import jax.numpy as jnp
from jax import lax
import jax.experimental.pallas as pl
import jax.experimental.pallas.tpu as pltpu

f32 = jnp.float32
bf16 = jnp.bfloat16

C = 128
T = 512
RC = 32
PR = 64


def _dft_consts(c):
    n = np.arange(c, dtype=np.float64)
    f = np.arange(c, dtype=np.float64)
    th = np.pi * np.outer(2 * f + 1, n) / (2 * c)
    fm = np.concatenate([np.cos(th), -np.sin(th)], 0)
    gm = np.concatenate([np.cos(th.T), -np.sin(th.T)], 1) / c
    return fm.T, gm.T


def _schedule(nt, ns):
    tab = []
    for t in range(nt):
        for j in range(2 * t + 2):
            tab.append((t, j))
    per = len(tab) // ns
    assert per * ns == len(tab) and per % 2 == 0
    bpt = 2 * nt // ns
    for n, (t, j) in enumerate(tab):
        step = n // per
        assert j < bpt * min(step + 2, ns)
        assert step <= (2 * t) // bpt
        assert n % 2 == 1 or tab[n + 1] == (t, j + 1)
    return np.array(tab, dtype=np.int32).T.copy(), per


def _kernel(tab_ref, q_ref, k0_ref, v0_ref, k_ref, v_ref, sk_ref, sd_ref, f_ref, g_ref,
            ssmk_hbm, w1_hbm, w2t_hbm, o_ref,
            xs_ref, ks_ref, pacc_ref, kvb_ref, kext_ref, w1t_ref, tap_ref, kvd_ref,
            ssmk_ref, w1_ref, w2t_ref, sems, *, nb, d, ns, per):
    s = pl.program_id(0)

    cp_ssmk = pltpu.make_async_copy(ssmk_hbm, ssmk_ref, sems.at[0])
    cp_w1 = pltpu.make_async_copy(w1_hbm, w1_ref, sems.at[1])
    cp_w2 = pltpu.make_async_copy(w2t_hbm, w2t_ref, sems.at[2])

    def process_block(b, kr, vr):
        for c in range(d // PR):
            rows = slice(c * PR, (c + 1) * PR)
            kb = kr[rows, :]
            ku = pltpu.bitcast(
                jnp.concatenate([kext_ref[rows, :], kb], axis=1), jnp.uint32)
            kext_ref[rows, :] = kb[:, T - C:]
            kshift = kb.astype(f32) * jnp.concatenate(
                [tap_ref[0, rows, :]] * (T // C), axis=1)
            for l in range(1, 4):
                sh = pltpu.bitcast(pltpu.roll(ku, l, 1)[:, C:], bf16).astype(f32)
                kshift = kshift + sh * jnp.concatenate(
                    [tap_ref[l, rows, :]] * (T // C), axis=1)
            kv = kshift * vr[rows, :].astype(f32)
            kvd_ref[b, rows, :] = kv * jnp.concatenate(
                [tap_ref[4, rows, :]] * (T // C), axis=1)
            kvb_ref[rows, :] = kv.astype(bf16)
        for e in range(T // C):
            xe = jnp.dot(kvb_ref[:, e * C:(e + 1) * C], f_ref[...],
                         preferred_element_type=f32)
            xs_ref[(T // C) * b + e, :, 0:2 * C] = xe
            xs_ref[(T // C) * b + e, :, 2 * C:3 * C] = xe[:, :C] + xe[:, C:]

    @pl.when(s == 0)
    def _():
        cp_ssmk.start()
        cp_w1.start()
        cp_w2.start()
        kext_ref[...] = jnp.zeros_like(kext_ref)
        pacc_ref[...] = jnp.zeros_like(pacc_ref)
        sk = jnp.transpose(sk_ref[...].astype(f32))
        for l in range(4):
            tap_ref[l] = jnp.broadcast_to(sk[:, l:l + 1], (d, C))
        sdc = jnp.transpose(sd_ref[...].astype(f32).reshape(1, d))
        tap_ref[4] = jnp.broadcast_to(sdc, (d, C))
        process_block(0, k0_ref, v0_ref)

    @pl.when(s < ns - 1)
    def _():
        process_block(s + 1, k_ref, v_ref)

    @pl.when(s == 0)
    def _():
        cp_ssmk.wait()
        fm = f_ref[...]
        ks_ref[0] = jnp.zeros((d, 3 * C), f32)
        lane = lax.broadcasted_iota(jnp.int32, (1, C), 1)
        sig = jnp.where(lane % 2 == 0, 1.0, -1.0).astype(f32)
        pr = pi = None
        for m in range(nb):
            kbm = ssmk_ref[:, m * C:(m + 1) * C]
            km = jnp.dot(kbm, fm, preferred_element_type=f32)
            kr, ki = km[:, :C], km[:, C:]
            if m == 0:
                ar, ai = kr, ki
            else:
                ar = kr - sig * pi
                ai = ki + sig * pr
            ks_ref[m + 1, :, 0:C] = ar
            ks_ref[m + 1, :, C:2 * C] = ai - ar
            ks_ref[m + 1, :, 2 * C:3 * C] = ar + ai
            pr, pi = kr, ki
        cp_w1.wait()
        w1t_ref[...] = w1_ref[...].T
        cp_w2.wait()

    x = q_ref[...].astype(f32)
    mu = jnp.mean(x, axis=0, keepdims=True)
    xc = x - mu
    var = jnp.mean(xc * xc, axis=0, keepdims=True)
    xn = xc * lax.rsqrt(var + 1e-5)
    xnb = xn.astype(bf16)

    for u in range(0, per, 2):
        n = s * per + u
        t = tab_ref[0, n]
        j = tab_ref[1, n]
        m0 = 2 * t - j + 1
        for rc in range(d // RC):
            rows = slice(rc * RC, (rc + 1) * RC)
            xa = [xs_ref[j, rows, e * C:(e + 1) * C] for e in range(3)]
            xb = [xs_ref[j + 1, rows, e * C:(e + 1) * C] for e in range(3)]
            km = [ks_ref[m0 - 1, rows, e * C:(e + 1) * C] for e in range(3)]
            k0 = [ks_ref[m0, rows, e * C:(e + 1) * C] for e in range(3)]
            kp = [ks_ref[m0 + 1, rows, e * C:(e + 1) * C] for e in range(3)]
            for e, (xe, ke) in enumerate(((2, 0), (1, 2), (0, 1))):
                cols = slice(e * C, (e + 1) * C)
                pacc_ref[2 * t, rows, cols] += xa[xe] * k0[ke] + xb[xe] * km[ke]
                pacc_ref[2 * t + 1, rows, cols] += xa[xe] * kp[ke] + xb[xe] * k0[ke]

    h = jnp.dot(w1t_ref[...], xnb, preferred_element_type=f32)
    hh = 0.5 * h
    h = (hh + hh * jnp.tanh(hh)).astype(bf16)
    ffn = jnp.dot(w2t_ref[...], h, preferred_element_type=f32)

    ys = []
    for e in range(T // C):
        a1 = pacc_ref[(T // C) * s + e, :, 0:C]
        a2 = pacc_ref[(T // C) * s + e, :, C:2 * C]
        a3 = pacc_ref[(T // C) * s + e, :, 2 * C:3 * C]
        pe = jnp.concatenate([a1 - a2, a1 + a3], axis=1).astype(bf16)
        ys.append(jnp.dot(pe, g_ref[...], preferred_element_type=f32))
    y = jnp.concatenate(ys, axis=1) + kvd_ref[s]
    o_ref[...] = (x + xn * y + ffn).astype(o_ref.dtype)


@jax.jit
def pallas_parallel_sum__ssm_conv_h3__dense_activation_silu__prompt_kernel(
    A_q: jax.Array,
    A_k: jax.Array,
    A_v: jax.Array,
    A_shift_k: jax.Array,
    A_ssm_k: jax.Array,
    A_ssm_D: jax.Array,
    B_x: jax.Array,
    B_w1: jax.Array,
    B_w2: jax.Array,
):
    B, S, D = A_q.shape
    F = B_w1.shape[1]
    nb = S // C
    ns = S // T
    q = A_q.reshape(S, D).T
    k = A_k.reshape(S, D).T
    v = A_v.reshape(S, D).T
    sd = A_ssm_D
    sk = A_shift_k.T
    w2t = B_w2.T
    fm, g = _dft_consts(C)
    fm = jnp.asarray(fm, dtype=bf16)
    g = jnp.asarray(g, dtype=bf16)
    tab, per = _schedule(nb // 2, ns)
    tab = jnp.asarray(tab)

    full = lambda shape: pl.BlockSpec(shape, lambda i: (0,) * len(shape))
    col = pl.BlockSpec((D, T), lambda i: (0, i))
    col0 = pl.BlockSpec((D, T), lambda i: (0, 0))
    coln = pl.BlockSpec((D, T), lambda i: (0, jnp.minimum(i + 1, ns - 1)))
    hbm = pl.BlockSpec(memory_space=pl.ANY)
    out = pl.pallas_call(
        functools.partial(_kernel, nb=nb, d=D, ns=ns, per=per),
        grid=(ns,),
        in_specs=[pl.BlockSpec(memory_space=pltpu.SMEM),
                  col, col0, col0, coln, coln, full((4, D)), full((D,)),
                  full((C, 2 * C)), full((2 * C, C)), hbm, hbm, hbm],
        out_specs=col,
        out_shape=jax.ShapeDtypeStruct((D, S), A_q.dtype),
        scratch_shapes=[
            pltpu.VMEM((nb, D, 3 * C), f32),
            pltpu.VMEM((nb + 1, D, 3 * C), f32),
            pltpu.VMEM((nb, D, 3 * C), f32),
            pltpu.VMEM((D, T), bf16),
            pltpu.VMEM((D, C), bf16),
            pltpu.VMEM((F, D), bf16),
            pltpu.VMEM((5, D, C), f32),
            pltpu.VMEM((ns, D, T), f32),
            pltpu.VMEM((D, S), bf16),
            pltpu.VMEM((D, F), bf16),
            pltpu.VMEM((D, F), bf16),
            pltpu.SemaphoreType.DMA((3,)),
        ],
        compiler_params=pltpu.CompilerParams(
            dimension_semantics=("arbitrary",),
            vmem_limit_bytes=100 * 1024 * 1024,
        ),
    )(tab, q, k, v, k, v, sk, sd, fm, g, A_ssm_k, B_w1, w2t)
    return out.T.reshape(B, S, D)
```
